```python
import jax
import jax.numpy as jnp

def _softmax(x, axis=-1):
    return jax.nn.softmax(x, axis=axis)
def _gelu(x):
    return jax.nn.gelu(x, approximate=True)
def _silu(x):
    return jax.nn.silu(x)
def _sigmoid(x):
    return jax.nn.sigmoid(x)
def _layernorm(x, axis=-1, eps=1e-5):
    m = jnp.mean(x, axis=axis, keepdims=True)
    v = jnp.var(x, axis=axis, keepdims=True)
    return (x - m) / jnp.sqrt(v + eps)
def _scatter_add(tgt, idx, src, axis=0):
    return tgt.at[idx].add(src)
def _segment_sum(src, seg, n):
    return jax.ops.segment_sum(src, seg, n)
class _Rng:
    def __init__(self, key):
        self._k = key
    def _next(self):
        self._k, sub = jax.random.split(self._k)
        return sub
    def normal(self, shape):
        return jax.random.normal(self._next(), shape, dtype=jnp.bfloat16)
    def randint(self, lo, hi, shape):
        return jax.random.randint(self._next(), shape, lo, hi, dtype=jnp.int32)
    def uniform(self, shape, lo=0.0, hi=1.0):
        return jax.random.uniform(self._next(), shape, jnp.bfloat16, lo, hi)
    def permutation(self, n):
        return jax.random.permutation(self._next(), n)


kernel_name = 'concat_heads__spectral_gfnet__compressed_kv_cla__prompt'

def setup_inputs():
    _rng = _Rng(jax.random.key(int.from_bytes(__import__("os").urandom(4), "little")))
    _w = (lambda a: (lambda t: t.astype(jnp.bfloat16) if jnp.issubdtype(t.dtype, jnp.floating) else t)(jnp.asarray(a)))
    def _A_setup():
        B, S, D = 1, 2048, 448
        Df = D // 2 + 1
        return {
            "x": _w((lambda *s: _rng.normal(s) * 0.05)(B, S, D)),
            "w_r": _w((lambda *s: _rng.normal(s) * 0.05)(S, Df) * 0.02),
            "w_i": _w((lambda *s: _rng.normal(s) * 0.05)(S, Df) * 0.02),
        }
    _A_in = _A_setup()

    def _B_setup():
        B, H, Sq, Sk, D, M = 1, 16, 2048, 2048, 256, 448
        Dc = 4 * D
        return {
            "x": _w((lambda *s: _rng.normal(s) * 0.05)(B, Sq, M)),
            "c_kv": _w((lambda *s: _rng.normal(s) * 0.05)(B, Sk, Dc)),
            "w_q": _w((lambda *s: _rng.normal(s) * 0.05)(M, H, D) * (M ** -0.5)),
            "w_uk": _w((lambda *s: _rng.normal(s) * 0.05)(Dc, H, D) * (Dc ** -0.5)),
            "w_uv": _w((lambda *s: _rng.normal(s) * 0.05)(Dc, H, D) * (Dc ** -0.5)),
            "w_o": _w((lambda *s: _rng.normal(s) * 0.05)(H, D, M) * ((H * D) ** -0.5)),
        }
    _B_in = _B_setup()

    return {
        "A_x": _A_in["x"],
        "A_w_r": _A_in["w_r"],
        "A_w_i": _A_in["w_i"],
        "B_x": _B_in["x"],
        "B_c_kv": _B_in["c_kv"],
        "B_w_q": _B_in["w_q"],
        "B_w_uk": _B_in["w_uk"],
        "B_w_uv": _B_in["w_uv"],
        "B_w_o": _B_in["w_o"],
    }

def reference(A_x, A_w_r, A_w_i, B_x, B_c_kv, B_w_q, B_w_uk, B_w_uv, B_w_o):
    def _A_ref(x, w_r, w_i):
        B, S, D = x.shape
        X = (lambda x, axes=(-2,-1): jnp.fft.rfft2(x.astype(jnp.float32), axes=axes))(x, axes=(-2, -1))
        W = w_r + 1j * w_i
        X = X * W
        y = (lambda x, s, axes=(-2,-1): jnp.fft.irfft2(x, s=s, axes=axes).astype(jnp.bfloat16))(X, (S, D), axes=(-2, -1))
        return y

    def _B_ref(x, c_kv, w_q, w_uk, w_uv, w_o):
        B, Sq, M = x.shape[0], x.shape[1], x.shape[2]
        Sk = c_kv.shape[1]
        H, D = w_q.shape[1], w_q.shape[2]
        q = jnp.einsum("bqm,mhd->bhqd", x, w_q)
        k = jnp.einsum("bkc,chd->bhkd", c_kv, w_uk)
        v = jnp.einsum("bkc,chd->bhkd", c_kv, w_uv)
        scores = jnp.einsum("bhqd,bhkd->bhqk", q, k) * (D ** -0.5)
        off = Sk - Sq
        qi = jnp.arange(Sq)[:, None]
        kj = jnp.arange(Sk)[None, :]
        cmask = kj <= (qi + off)
        scores = jnp.where(cmask[None, None], scores, -1e9)
        p = _softmax(scores, axis=-1)
        ctx = jnp.einsum("bhqk,bhkd->bhqd", p, v)
        return jnp.einsum("bhqd,hdm->bqm", ctx, w_o)

    a = _A_ref(A_x, A_w_r, A_w_i)
    b = _B_ref(B_x, B_c_kv, B_w_q, B_w_uk, B_w_uv, B_w_o)
    return jnp.concatenate([a, b], axis=-1)
```

```python
import functools
import math

import jax
import jax.experimental.pallas as pl
import jax.experimental.pallas.tpu as pltpu
import jax.numpy as jnp
import numpy as np
from jax import lax

bf16 = jnp.bfloat16
f32 = jnp.float32
u32 = jnp.uint32
NT = (((1,), (1,)), ((), ()))

SEQ = 2048
DM = 448
NF = 225
H = 16
DH = 256
DC = 1024
BQ = 256
NB = SEQ // BQ
N1 = 32
N2 = 64
HI16 = np.uint32(0xFFFF0000)


def _to_bf16(a):
    return np.asarray(a, dtype=np.float32).astype(jnp.bfloat16)


@functools.lru_cache(maxsize=None)
def _dft_constants():
    half = DM // 2
    m = np.arange(half, dtype=np.float64)
    fd = np.zeros((2, 256, 256), np.float64)
    gd = np.zeros((2, 256, 256), np.float64)
    for par in range(2):
        ks = np.arange(par, NF, 2, dtype=np.float64)
        ang = 2.0 * np.pi * np.outer(m, ks) / DM
        nk = len(ks)
        fd[par, :half, :nk] = np.cos(ang)
        fd[par, :half, 128:128 + nk] = -np.sin(ang)
        wgt = np.full(nk, 2.0)
        wgt[(ks == 0) | (ks == half)] = 1.0
        gd[par, :nk, :half] = (np.cos(ang) * wgt / DM).T
        snk = -np.sin(ang) * wgt / DM
        snk[:, (ks == 0) | (ks == half)] = 0.0
        gd[par, 128:128 + nk, :half] = snk.T
    b = np.arange(N2, dtype=np.float64)
    sf = np.zeros((N1, 128, 128), np.float64)
    si = np.zeros((N1, 128, 128), np.float64)
    for f1 in range(N1):
        mat = np.exp(-2j * np.pi * (np.outer(b, b) / N2 + b[None, :] * f1 / SEQ))
        sf[f1] = np.block([[mat.real, -mat.imag], [mat.imag, mat.real]])
        inv = np.conj(mat).T / SEQ
        si[f1] = np.block([[inv.real, -inv.imag], [inv.imag, inv.real]])
    return _to_bf16(fd), _to_bf16(sf), _to_bf16(si), _to_bf16(gd)


def _lo(v):
    return pltpu.bitcast(v << 16, f32)


def _hi(v):
    return pltpu.bitcast(v & HI16, f32)


def _cmul_const(z, w):
    re, im = z
    c, s = w.real, w.imag
    if abs(s) < 1e-12:
        return (re, im) if c > 0 else (-re, -im)
    if abs(c) < 1e-12:
        return (-im, re) if s > 0 else (im, -re)
    if abs(abs(c) - abs(s)) < 1e-12:
        if c * s > 0:
            return ((re - im) * c, (re + im) * c)
        return ((re + im) * c, (im - re) * c)
    return (re * c - im * s, re * s + im * c)


def _fft(xs, sign):
    n = len(xs)
    if n == 1:
        return xs
    ev = _fft(xs[0::2], sign)
    od = _fft(xs[1::2], sign)
    out = [None] * n
    for k in range(n // 2):
        w = complex(math.cos(2 * math.pi * k / n), sign * math.sin(2 * math.pi * k / n))
        if 4 * k == n:
            tr, ti = od[k]
            if sign < 0:
                out[k] = (ev[k][0] + ti, ev[k][1] - tr)
                out[k + n // 2] = (ev[k][0] - ti, ev[k][1] + tr)
            else:
                out[k] = (ev[k][0] - ti, ev[k][1] + tr)
                out[k + n // 2] = (ev[k][0] + ti, ev[k][1] - tr)
            continue
        tr, ti = _cmul_const(od[k], w)
        out[k] = (ev[k][0] + tr, ev[k][1] + ti)
        out[k + n // 2] = (ev[k][0] - tr, ev[k][1] - ti)
    return out


def _radix32(ure, uim, rows, sign):
    for q in range(4):
        xs = [(ure[rows(4 * p + q), :], uim[rows(4 * p + q), :]) for p in range(8)]
        ys = _fft(xs, sign)
        for u in range(8):
            w = complex(math.cos(2 * math.pi * q * u / 32), sign * math.sin(2 * math.pi * q * u / 32))
            tr, ti = _cmul_const(ys[u], w)
            ure[rows(4 * u + q), :] = tr
            uim[rows(4 * u + q), :] = ti
    for u in range(8):
        xs = [(ure[rows(4 * u + q), :], uim[rows(4 * u + q), :]) for q in range(4)]
        ys = _fft(xs, sign)
        for v in range(4):
            ure[rows(4 * u + v), :] = ys[v][0]
            uim[rows(4 * u + v), :] = ys[v][1]


def _radix32_inv(ure, uim, rows, sign):
    for u in range(8):
        xs = [(ure[rows(4 * u + v), :], uim[rows(4 * u + v), :]) for v in range(4)]
        ys = _fft(xs, sign)
        for q in range(4):
            w = complex(math.cos(2 * math.pi * q * u / 32), sign * math.sin(2 * math.pi * q * u / 32))
            tr, ti = _cmul_const(ys[q], w)
            ure[rows(4 * u + q), :] = tr
            uim[rows(4 * u + q), :] = ti
    for q in range(4):
        xs = [(ure[rows(4 * u + q), :], uim[rows(4 * u + q), :]) for u in range(8)]
        ys = _fft(xs, sign)
        for p in range(8):
            ure[rows(4 * p + q), :] = ys[p][0]
            uim[rows(4 * p + q), :] = ys[p][1]


def _tri():
    r = lax.broadcasted_iota(jnp.int32, (128, 128), 0)
    c = lax.broadcasted_iota(jnp.int32, (128, 128), 1)
    return c <= r


def _scores(q, k_ref, r0):
    n = r0 + 128
    s = lax.dot_general(q, k_ref[0:n, :], NT, preferred_element_type=f32)
    se = lax.dot_general(q[128:], k_ref[n:n + 128, :], NT, preferred_element_type=f32)
    return s, se


def _softmax(s, se, r0):
    tri = _tri()
    se = jnp.where(tri, se, -1e9)
    su, sl = s[:128], s[128:]
    sd = jnp.where(tri, su[:, r0:], -1e9)
    su = jnp.concatenate([su[:, :r0], sd], axis=1) if r0 > 0 else sd
    mu = jnp.max(su, axis=-1, keepdims=True)
    ml = jnp.maximum(jnp.max(sl, axis=-1, keepdims=True), jnp.max(se, axis=-1, keepdims=True))
    pu = jnp.exp2(su - mu)
    pl_ = jnp.exp2(sl - ml)
    pe = jnp.exp2(se - ml)
    lu = jnp.sum(pu, axis=-1, keepdims=True)
    ll = jnp.sum(pl_, axis=-1, keepdims=True) + jnp.sum(pe, axis=-1, keepdims=True)
    p = jnp.concatenate([pu, pl_], axis=0).astype(bf16)
    return p, pe.astype(bf16), lu, ll


def _context(p, pe, lu, ll, v_ref, r0):
    n = r0 + 128
    o = jnp.dot(p, v_ref[0:n, :], preferred_element_type=f32)
    oe = jnp.dot(pe, v_ref[n:n + 128, :], preferred_element_type=f32)
    return jnp.concatenate([o[:128] / lu, (o[128:] + oe) / ll], axis=0).astype(bf16)


def _head_schedule():
    s = [("QK", 0)]
    for i in range(NB):
        if i + 1 < NB:
            s.append(("QK", i + 1))
        s.append(("PV", i))
        if i > 0:
            s.append(("O", i - 1))
        s.append(("KV", i))
    s.append(("O", NB - 1))
    return s


(S_XA, S_FD, S_SF, S_WR, S_WI, S_SI, S_GD, S_XB, S_CKV, S_WO) = range(10)
S_WQ = 10
S_UK = S_WQ + 8
S_UV = S_UK + 8
S_OUT = S_UV + 8
N_SEM = S_OUT + NB


def _kernel(
    xa_h, wr_h, wi_h, xb_h, ckv_h, wq_h, uk_h, uv_h, wo_h, fd_h, sf_h, si_h, gd_h,
    out_h,
    xa_v, wr_v, wi_v, xb_v, ckv_v, wq_v, uk_v, uv_v, wo_v, fd_v, sf_v, si_v, gd_v,
    xf_v, ure, uim, wn_re, wn_im, x_v, wqp_v, q_v, k_v, v_v, wkv_v, acc_v, out_v, sem,
):
    cp = pltpu.make_async_copy
    wq_u, uk_u, uv_u = wq_h.bitcast(u32), uk_h.bitcast(u32), uv_h.bitcast(u32)
    c_xa = cp(xa_h, xa_v, sem.at[S_XA])
    c_fd = cp(fd_h, fd_v, sem.at[S_FD])
    c_sf = cp(sf_h, sf_v, sem.at[S_SF])
    c_wr = cp(wr_h, wr_v, sem.at[S_WR])
    c_wi = cp(wi_h, wi_v, sem.at[S_WI])
    c_si = cp(si_h, si_v, sem.at[S_SI])
    c_gd = cp(gd_h, gd_v, sem.at[S_GD])
    c_xb = cp(xb_h, xb_v, sem.at[S_XB])
    c_ckv = cp(ckv_h, ckv_v, sem.at[S_CKV])
    c_wo = cp(wo_h, wo_v, sem.at[S_WO])
    c_wq = [cp(wq_u.at[:, j, :], wq_v.at[j], sem.at[S_WQ + j]) for j in range(8)]
    c_uk = [cp(uk_u.at[:, j, :], uk_v.at[j], sem.at[S_UK + j]) for j in range(8)]
    c_uv = [cp(uv_u.at[:, j, :], uv_v.at[j], sem.at[S_UV + j]) for j in range(8)]
    for c in [c_xa, c_fd, c_wr, c_wi, c_sf, c_si, c_gd, c_xb] + c_wq + [c_ckv, c_uk[0], c_uv[0], c_wo]:
        c.start()
    for j in range(1, 8):
        c_uk[j].start()
        c_uv[j].start()

    half = DM // 2
    c_xa.wait()
    c_fd.wait()
    for par in range(2):
        for cb in range(SEQ // 256):
            cols = slice(cb * 256, (cb + 1) * 256)
            x0 = xa_v[0:half, cols].astype(f32)
            x1 = xa_v[half:DM, cols].astype(f32)
            xf = (x0 + x1 if par == 0 else x0 - x1).astype(bf16)
            xf = jnp.concatenate([xf, jnp.zeros((256 - half, 256), bf16)], axis=0)
            xf_v[par, cols, :] = xf.T
    for par in range(2):
        u = jnp.dot(xf_v[par], fd_v[par], preferred_element_type=f32)
        ure[:, par * 128:(par + 1) * 128] = u[:, :128]
        uim[:, par * 128:(par + 1) * 128] = u[:, 128:]

    def fwd_rows(r, carry):
        r8 = pl.multiple_of(r * 8, 8)
        _radix32(ure, uim, lambda blk: pl.ds(blk * N2 + r8, 8), -1)
        return carry

    lax.fori_loop(0, N2 // 8, fwd_rows, 0)

    c_wr.wait()
    c_wi.wait()
    for w_v, wn in ((wr_v, wn_re), (wi_v, wn_im)):
        for cb in range(SEQ // 256):
            cols = slice(cb * 256, (cb + 1) * 256)
            wu = pltpu.bitcast(w_v[0:half, cols], u32)
            last = w_v[half:NF, cols].astype(f32)
            row0 = lax.broadcasted_iota(jnp.int32, (16, 256), 0) == 0
            tail = jnp.where(row0, jnp.broadcast_to(last, (16, 256)), 0.0)
            we = jnp.concatenate([_lo(wu), tail], axis=0).astype(bf16)
            wo = jnp.concatenate([_hi(wu), jnp.zeros((16, 256), f32)], axis=0).astype(bf16)
            wn[0, cols, :] = we.T.astype(f32)
            wn[1, cols, :] = wo.T.astype(f32)

    c_sf.wait()
    c_si.wait()
    for f1 in range(N1):
        slot = 4 * (f1 % 8) + f1 // 8
        rows = slice(slot * N2, (slot + 1) * N2)
        y = jnp.concatenate([ure[rows, :], uim[rows, :]], axis=0).astype(bf16)
        xs = jnp.dot(sf_v[f1], y, preferred_element_type=f32)
        xr, xi = xs[:N2], xs[N2:]
        fr = pl.ds(f1, N2, stride=N1)
        wr = jnp.concatenate([wn_re[0, fr, :], wn_re[1, fr, :]], axis=1)
        wi = jnp.concatenate([wn_im[0, fr, :], wn_im[1, fr, :]], axis=1)
        xw = jnp.concatenate([xr * wr - xi * wi, xr * wi + xi * wr], axis=0).astype(bf16)
        z = jnp.dot(si_v[f1], xw, preferred_element_type=f32)
        ure[rows, :] = z[:N2]
        uim[rows, :] = z[N2:]

    def inv_rows(r, carry):
        r8 = pl.multiple_of(r * 8, 8)
        _radix32_inv(ure, uim, lambda blk: pl.ds(blk * N2 + r8, 8), 1)
        return carry

    lax.fori_loop(0, N2 // 8, inv_rows, 0)

    c_gd.wait()
    for rb in range(SEQ // 512):
        rows = slice(rb * 512, (rb + 1) * 512)
        ze = jnp.concatenate([ure[rows, 0:128], uim[rows, 0:128]], axis=1).astype(bf16)
        zo = jnp.concatenate([ure[rows, 128:256], uim[rows, 128:256]], axis=1).astype(bf16)
        ye = jnp.dot(ze, gd_v[0], preferred_element_type=f32)[:, :half]
        yo = jnp.dot(zo, gd_v[1], preferred_element_type=f32)[:, :half]
        out_v[rows, 0:half] = (ye + yo).astype(bf16)
        out_v[rows, half:DM] = (ye - yo).astype(bf16)

    c_xb.wait()
    x_v[:, DM:512] = jnp.zeros((SEQ, 512 - DM), bf16)
    for cb in range(SEQ // 256):
        cols = slice(cb * 256, (cb + 1) * 256)
        x_v[cols, 0:DM] = xb_v[:, cols].T
    wqp_v[DM:512, :] = jnp.zeros((512 - DM, 512), bf16)
    acc_v[...] = jnp.zeros(acc_v.shape, f32)
    for c in c_wq:
        c.wait()

    qscale = np.float32(DH ** -0.5 * math.log2(math.e))

    def q_pair(j, carry):
        w = wq_v[j]
        wqp_v[0:DM, 0:DH] = _lo(w).astype(bf16)
        wqp_v[0:DM, DH:2 * DH] = _hi(w).astype(bf16)
        q = jnp.dot(x_v[...], wqp_v[...], preferred_element_type=f32) * qscale
        q_v[j] = q.astype(bf16)
        return carry

    lax.fori_loop(0, 8, q_pair, 0)

    def relayout(head, slot):
        j = head // 2
        sh = ((1 - head % 2) * 16).astype(u32)
        for c0 in range(0, DC, 128):
            for n, src in enumerate((uk_v, uv_v)):
                w = src[j, c0:c0 + 128, :]
                wkv_v[slot, c0:c0 + 128, n * DH:(n + 1) * DH] = pltpu.bitcast((w << sh) & HI16, f32).astype(bf16)

    def kv_rows(slot, r0, r1):
        kv = jnp.dot(ckv_v[r0:r1, :], wkv_v[slot], preferred_element_type=f32)
        k_v[slot, r0:r1, :] = kv[:, :DH].astype(bf16)
        v_v[slot, r0:r1, :] = kv[:, DH:].astype(bf16)

    c_ckv.wait()
    c_uk[0].wait()
    c_uv[0].wait()
    relayout(jnp.int32(0), 0)

    def kv0(i, carry):
        r0 = pl.multiple_of(i * 512, 512)
        kv = jnp.dot(ckv_v[pl.ds(r0, 512), :], wkv_v[0], preferred_element_type=f32)
        k_v[0, pl.ds(r0, 512), :] = kv[:, :DH].astype(bf16)
        v_v[0, pl.ds(r0, 512), :] = kv[:, DH:].astype(bf16)
        return carry

    lax.fori_loop(0, SEQ // 512, kv0, 0)

    c_wo.wait()
    for j in range(1, 8):
        c_uk[j].wait()
        c_uv[j].wait()

    def head(h, last):
        cur = h % 2
        nxt = 1 - cur
        kc, vc = k_v.at[cur], v_v.at[cur]
        qcol = pl.ds(pl.multiple_of((h % 2) * DH, DH), DH) if not last else (h % 2) * DH
        if not last:
            relayout(h + 1, nxt)
        ss, os_ = {}, {}
        for op, i in _head_schedule():
            r0 = i * BQ
            if op == "QK":
                qc = qcol if not last else slice(qcol, qcol + DH)
                ss[i] = _scores(q_v[h // 2, r0:r0 + BQ, qc], kc, r0)
            elif op == "PV":
                os_[i] = _context(*_softmax(*ss.pop(i), r0), vc, r0)
            elif op == "KV":
                if not last:
                    kv_rows(nxt, r0, r0 + BQ)
            elif op == "O":
                t = lax.dot_general(wo_v[h], os_.pop(i), NT, preferred_element_type=f32)
                if not last:
                    acc_v[64:512, r0:r0 + BQ] += t
                else:
                    bt = jnp.concatenate([jnp.zeros((64, BQ), f32), acc_v[64:512, r0:r0 + BQ] + t], axis=0)
                    b = bt.astype(bf16).T
                    lane = lax.broadcasted_iota(jnp.int32, (BQ, 128), 1)
                    a_tail = jnp.where(lane < 64, out_v[r0:r0 + BQ, 384:512], jnp.zeros((BQ, 128), bf16))
                    out_v[r0:r0 + BQ, 384:512] = jnp.where(lane < 64, a_tail, b[:, :128])
                    out_v[r0:r0 + BQ, 512:896] = b[:, 128:]
                    cp(out_v.at[r0:r0 + BQ], out_h.at[r0:r0 + BQ], sem.at[S_OUT + i]).start()

    def head_loop(h, carry):
        head(h, False)
        return carry

    lax.fori_loop(0, H - 1, head_loop, 0)
    head(H - 1, True)
    for i in range(NB):
        r0 = i * BQ
        cp(out_v.at[r0:r0 + BQ], out_h.at[r0:r0 + BQ], sem.at[S_OUT + i]).wait()


@jax.jit
def pallas_concat_heads__spectral_gfnet__compressed_kv_cla__prompt_kernel(
    A_x: jax.Array,
    A_w_r: jax.Array,
    A_w_i: jax.Array,
    B_x: jax.Array,
    B_c_kv: jax.Array,
    B_w_q: jax.Array,
    B_w_uk: jax.Array,
    B_w_uv: jax.Array,
    B_w_o: jax.Array,
):
    fd, sf, si, gd = _dft_constants()
    args = (
        A_x.reshape(SEQ, DM).T,
        A_w_r.T,
        A_w_i.T,
        B_x.reshape(SEQ, DM).T,
        B_c_kv.reshape(SEQ, DC),
        B_w_q,
        B_w_uk,
        B_w_uv,
        jnp.transpose(B_w_o, (0, 2, 1)),
        fd, sf, si, gd,
    )
    vm = pltpu.VMEM
    scratch = [
        vm((DM, SEQ), bf16),
        vm((NF, SEQ), bf16),
        vm((NF, SEQ), bf16),
        vm((DM, SEQ), bf16),
        vm((SEQ, DC), bf16),
        vm((8, DM, DH), u32),
        vm((8, DC, DH), u32),
        vm((8, DC, DH), u32),
        vm((H, DM, DH), bf16),
        vm((2, 256, 256), bf16),
        vm((N1, 128, 128), bf16),
        vm((N1, 128, 128), bf16),
        vm((2, 256, 256), bf16),
        vm((2, SEQ, 256), bf16),
        vm((SEQ, 256), f32),
        vm((SEQ, 256), f32),
        vm((2, SEQ, 128), f32),
        vm((2, SEQ, 128), f32),
        vm((SEQ, 512), bf16),
        vm((512, 512), bf16),
        vm((8, SEQ, 2 * DH), bf16),
        vm((2, SEQ, DH), bf16),
        vm((2, SEQ, DH), bf16),
        vm((2, DC, 2 * DH), bf16),
        vm((512, SEQ), f32),
        vm((SEQ, 2 * DM), bf16),
        pltpu.SemaphoreType.DMA((N_SEM,)),
    ]
    out = pl.pallas_call(
        _kernel,
        in_specs=[pl.BlockSpec(memory_space=pl.ANY)] * len(args),
        out_specs=pl.BlockSpec(memory_space=pl.ANY),
        out_shape=jax.ShapeDtypeStruct((SEQ, 2 * DM), bf16),
        scratch_shapes=scratch,
        compiler_params=pltpu.CompilerParams(vmem_limit_bytes=120 * 2**20),
    )(*args)
    return out.reshape(1, SEQ, 2 * DM)
```

```python
import functools
import math

import jax
import jax.experimental.pallas as pl
import jax.experimental.pallas.tpu as pltpu
import jax.numpy as jnp
import numpy as np
from jax import lax

bf16 = jnp.bfloat16
f32 = jnp.float32
u32 = jnp.uint32
NT = (((1,), (1,)), ((), ()))

SEQ = 2048
DM = 448
NF = 225
H = 16
DH = 256
DC = 1024
BQ = 256
NB = SEQ // BQ
N1 = 32
N2 = 64
WP = N1 + 1
HI16 = np.uint32(0xFFFF0000)


def _to_bf16(a):
    return np.asarray(a, dtype=np.float32).astype(jnp.bfloat16)


@functools.lru_cache(maxsize=None)
def _dft_constants():
    half = DM // 2
    m = np.arange(half, dtype=np.float64)
    fd = np.zeros((2, 256, 256), np.float64)
    gd = np.zeros((2, 256, 256), np.float64)
    for par in range(2):
        ks = np.arange(par, NF, 2, dtype=np.float64)
        ang = 2.0 * np.pi * np.outer(m, ks) / DM
        nk = len(ks)
        fd[par, :half, :nk] = np.cos(ang)
        fd[par, :half, 128:128 + nk] = -np.sin(ang)
        wgt = np.full(nk, 2.0)
        wgt[(ks == 0) | (ks == half)] = 1.0
        gd[par, :nk, :half] = (np.cos(ang) * wgt / DM).T
        snk = -np.sin(ang) * wgt / DM
        snk[:, (ks == 0) | (ks == half)] = 0.0
        gd[par, 128:128 + nk, :half] = snk.T
    b = np.arange(N2, dtype=np.float64)
    sf = np.zeros((N1, 128, 128), np.float64)
    si = np.zeros((N1, 128, 128), np.float64)
    for f1 in range(N1):
        mat = np.exp(-2j * np.pi * (np.outer(b, b) / N2 + b[None, :] * f1 / SEQ))
        sf[f1] = np.block([[mat.real, -mat.imag], [mat.imag, mat.real]])
        inv = np.conj(mat).T / SEQ
        si[f1] = np.block([[inv.real, -inv.imag], [inv.imag, inv.real]])
    return _to_bf16(fd), _to_bf16(sf), _to_bf16(si), _to_bf16(gd)


def _lo(v):
    return pltpu.bitcast(v << 16, f32)


def _hi(v):
    return pltpu.bitcast(v & HI16, f32)


def _cmul_const(z, w):
    re, im = z
    c, s = w.real, w.imag
    if abs(s) < 1e-12:
        return (re, im) if c > 0 else (-re, -im)
    if abs(c) < 1e-12:
        return (-im, re) if s > 0 else (im, -re)
    if abs(abs(c) - abs(s)) < 1e-12:
        if c * s > 0:
            return ((re - im) * c, (re + im) * c)
        return ((re + im) * c, (im - re) * c)
    return (re * c - im * s, re * s + im * c)


def _fft(xs, sign):
    n = len(xs)
    if n == 1:
        return xs
    ev = _fft(xs[0::2], sign)
    od = _fft(xs[1::2], sign)
    out = [None] * n
    for k in range(n // 2):
        w = complex(math.cos(2 * math.pi * k / n), sign * math.sin(2 * math.pi * k / n))
        if 4 * k == n:
            tr, ti = od[k]
            if sign < 0:
                out[k] = (ev[k][0] + ti, ev[k][1] - tr)
                out[k + n // 2] = (ev[k][0] - ti, ev[k][1] + tr)
            else:
                out[k] = (ev[k][0] - ti, ev[k][1] + tr)
                out[k + n // 2] = (ev[k][0] + ti, ev[k][1] - tr)
            continue
        tr, ti = _cmul_const(od[k], w)
        out[k] = (ev[k][0] + tr, ev[k][1] + ti)
        out[k + n // 2] = (ev[k][0] - tr, ev[k][1] - ti)
    return out


def _radix32(ure, uim, rows, sign):
    for q in range(4):
        xs = [(ure[rows(4 * p + q), :], uim[rows(4 * p + q), :]) for p in range(8)]
        ys = _fft(xs, sign)
        for u in range(8):
            w = complex(math.cos(2 * math.pi * q * u / 32), sign * math.sin(2 * math.pi * q * u / 32))
            tr, ti = _cmul_const(ys[u], w)
            ure[rows(4 * u + q), :] = tr
            uim[rows(4 * u + q), :] = ti
    for u in range(8):
        xs = [(ure[rows(4 * u + q), :], uim[rows(4 * u + q), :]) for q in range(4)]
        ys = _fft(xs, sign)
        for v in range(4):
            ure[rows(4 * u + v), :] = ys[v][0]
            uim[rows(4 * u + v), :] = ys[v][1]


def _radix32_inv(ure, uim, rows, sign):
    for u in range(8):
        xs = [(ure[rows(4 * u + v), :], uim[rows(4 * u + v), :]) for v in range(4)]
        ys = _fft(xs, sign)
        for q in range(4):
            w = complex(math.cos(2 * math.pi * q * u / 32), sign * math.sin(2 * math.pi * q * u / 32))
            tr, ti = _cmul_const(ys[q], w)
            ure[rows(4 * u + q), :] = tr
            uim[rows(4 * u + q), :] = ti
    for q in range(4):
        xs = [(ure[rows(4 * u + q), :], uim[rows(4 * u + q), :]) for u in range(8)]
        ys = _fft(xs, sign)
        for p in range(8):
            ure[rows(4 * p + q), :] = ys[p][0]
            uim[rows(4 * p + q), :] = ys[p][1]


def _tri():
    r = lax.broadcasted_iota(jnp.int32, (128, 128), 0)
    c = lax.broadcasted_iota(jnp.int32, (128, 128), 1)
    return c <= r


def _scores(q, k_ref, r0):
    n = r0 + 128
    s = lax.dot_general(q, k_ref[0:n, :], NT, preferred_element_type=f32)
    se = lax.dot_general(q[128:], k_ref[n:n + 128, :], NT, preferred_element_type=f32)
    return s, se


def _softmax(s, se, r0):
    tri = _tri()
    se = jnp.where(tri, se, -1e9)
    su, sl = s[:128], s[128:]
    sd = jnp.where(tri, su[:, r0:], -1e9)
    su = jnp.concatenate([su[:, :r0], sd], axis=1) if r0 > 0 else sd
    mu = jnp.max(su, axis=-1, keepdims=True)
    ml = jnp.maximum(jnp.max(sl, axis=-1, keepdims=True), jnp.max(se, axis=-1, keepdims=True))
    pu = jnp.exp2(su - mu)
    pl_ = jnp.exp2(sl - ml)
    pe = jnp.exp2(se - ml)
    lu = jnp.sum(pu, axis=-1, keepdims=True)
    ll = jnp.sum(pl_, axis=-1, keepdims=True) + jnp.sum(pe, axis=-1, keepdims=True)
    p = jnp.concatenate([pu, pl_], axis=0).astype(bf16)
    return p, pe.astype(bf16), lu, ll


def _context(p, pe, lu, ll, v_ref, r0):
    n = r0 + 128
    o = jnp.dot(p, v_ref[0:n, :], preferred_element_type=f32)
    oe = jnp.dot(pe, v_ref[n:n + 128, :], preferred_element_type=f32)
    return jnp.concatenate([o[:128] / lu, (o[128:] + oe) / ll], axis=0).astype(bf16)


def _head_schedule():
    s = [("CP", 0), ("QK", 0)]
    for i in range(NB):
        if i + 1 < NB:
            s += [("KV", i + 1), ("QK", i + 1)]
        else:
            s += [("RL", 0), ("KVN", 0)]
        s.append(("PV", i))
        if i > 0:
            s.append(("O", i - 1))
    s.append(("O", NB - 1))
    return s


(S_XA, S_FD, S_SF, S_WR, S_WI, S_SI, S_GD, S_XB, S_CKV, S_WO) = range(10)
S_WQ = 10
S_UK = S_WQ + 8
S_UV = S_UK + 8
S_OUT = S_UV + 8
N_SEM = S_OUT + NB


def _kernel(
    xa_h, wr_h, wi_h, xb_h, ckv_h, wq_h, uk_h, uv_h, wo_h, fd_h, sf_h, si_h, gd_h,
    out_h,
    xa_v, wr_v, wi_v, xb_v, ckv_v, wq_v, uk_v, uv_v, wo_v, fd_v, sf_v, si_v, gd_v,
    xf_v, u_v, wn_v, ye_v, x_v, wqp_v, q_v, k_v, v_v, kn_v, vn_v, wkv_v, acc_v, out_v, sem,
):
    cp = pltpu.make_async_copy
    wq_u, uk_u, uv_u = wq_h.bitcast(u32), uk_h.bitcast(u32), uv_h.bitcast(u32)
    c_xa = cp(xa_h, xa_v, sem.at[S_XA])
    c_fd = cp(fd_h, fd_v, sem.at[S_FD])
    c_sf = cp(sf_h, sf_v, sem.at[S_SF])
    c_wr = cp(wr_h, wr_v, sem.at[S_WR])
    c_wi = cp(wi_h, wi_v, sem.at[S_WI])
    c_si = cp(si_h, si_v, sem.at[S_SI])
    c_gd = cp(gd_h, gd_v, sem.at[S_GD])
    c_xb = cp(xb_h, xb_v, sem.at[S_XB])
    c_ckv = cp(ckv_h, ckv_v, sem.at[S_CKV])
    c_wo = cp(wo_h, wo_v, sem.at[S_WO])
    c_wq = [cp(wq_u.at[:, j, :], wq_v.at[j], sem.at[S_WQ + j]) for j in range(8)]
    c_uk = [cp(uk_u.at[:, j, :], uk_v.at[j], sem.at[S_UK + j]) for j in range(8)]
    c_uv = [cp(uv_u.at[:, j, :], uv_v.at[j], sem.at[S_UV + j]) for j in range(8)]
    for c in [c_xa, c_fd, c_wr, c_wi, c_sf, c_si, c_gd, c_xb] + c_wq + [c_ckv, c_uk[0], c_uv[0], c_wo]:
        c.start()
    for j in range(1, 8):
        c_uk[j].start()
        c_uv[j].start()

    half = DM // 2
    c_xa.wait()
    c_fd.wait()

    def a_fold(par):
        for cb in range(SEQ // 256):
            cols = slice(cb * 256, (cb + 1) * 256)
            x0 = xa_v[0:half, cols].astype(f32)
            x1 = xa_v[half:DM, cols].astype(f32)
            xf = (x0 + x1 if par == 0 else x0 - x1).astype(bf16)
            xf = jnp.concatenate([xf, jnp.zeros((256 - half, 256), bf16)], axis=0)
            xf_v[par, cols, :] = xf.T

    def a_dft(par):
        for rb in range(SEQ // 512):
            rows = slice(rb * 512, (rb + 1) * 512)
            u = jnp.dot(xf_v[par, rows, :], fd_v[par], preferred_element_type=f32)
            u_v[par, 0, rows, :] = u[:, :128]
            u_v[par, 1, rows, :] = u[:, 128:]

    def a_filter_prep(par):
        for ri, w_v in enumerate((wr_v, wi_v)):
            for cb in range(SEQ // 256):
                cols = slice(cb * 256, (cb + 1) * 256)
                wu = pltpu.bitcast(w_v[0:half, cols], u32)
                if par == 0:
                    last = w_v[half:NF, cols].astype(f32)
                    row0 = lax.broadcasted_iota(jnp.int32, (16, 256), 0) == 0
                    tail = jnp.where(row0, jnp.broadcast_to(last, (16, 256)), 0.0)
                    w = jnp.concatenate([_lo(wu), tail], axis=0).astype(bf16)
                else:
                    w = jnp.concatenate([_hi(wu), jnp.zeros((16, 256), f32)], axis=0).astype(bf16)
                wt = w.T.astype(f32)
                for g in range(256 // N1):
                    r0 = WP * (cb * (256 // N1) + g)
                    wn_v[par, ri, r0:r0 + N1, :] = wt[g * N1:(g + 1) * N1]

    def a_mid(par):
        for f1 in range(N1):
            slot = 4 * (f1 % 8) + f1 // 8
            rows = slice(slot * N2, (slot + 1) * N2)
            y = jnp.concatenate([u_v[par, 0, rows, :], u_v[par, 1, rows, :]], axis=0).astype(bf16)
            xs = jnp.dot(sf_v[f1], y, preferred_element_type=f32)
            xr, xi = xs[:N2], xs[N2:]
            fr = pl.ds(f1, N2, stride=WP)
            wr = wn_v[par, 0, fr, :]
            wi = wn_v[par, 1, fr, :]
            xw = jnp.concatenate([xr * wr - xi * wi, xr * wi + xi * wr], axis=0).astype(bf16)
            z = jnp.dot(si_v[f1], xw, preferred_element_type=f32)
            u_v[par, 0, rows, :] = z[:N2]
            u_v[par, 1, rows, :] = z[N2:]

    def a_radix(par, fn, sign):
        for r in range(0, N2, 8):
            fn(u_v.at[par, 0], u_v.at[par, 1], lambda blk: slice(blk * N2 + r, blk * N2 + r + 8), sign)

    def a_idft(par, rb):
        rows = slice(rb * 512, (rb + 1) * 512)
        z = jnp.concatenate([u_v[par, 0, rows, :], u_v[par, 1, rows, :]], axis=1).astype(bf16)
        return jnp.dot(z, gd_v[par], preferred_element_type=f32)[:, :half]

    for par in range(2):
        a_fold(par)
        a_dft(par)
    a_radix(0, _radix32, -1)
    for c in (c_wr, c_wi, c_sf, c_si):
        c.wait()
    a_filter_prep(0)
    a_filter_prep(1)
    a_radix(1, _radix32, -1)
    a_mid(0)
    a_radix(0, _radix32_inv, 1)
    a_mid(1)
    c_gd.wait()
    c_xb.wait()
    a_radix(1, _radix32_inv, 1)
    for cb in range(SEQ // 256):
        cols = slice(cb * 256, (cb + 1) * 256)
        x_v[cols, :] = jnp.concatenate([xb_v[:, cols], jnp.zeros((512 - DM, 256), bf16)], axis=0).T
    wqp_v[DM:512, :] = jnp.zeros((512 - DM, 512), bf16)
    for rb in range(SEQ // 512):
        ye_v[rb * 512:(rb + 1) * 512, :] = a_idft(0, rb)
    for rb in range(SEQ // 512):
        rows = slice(rb * 512, (rb + 1) * 512)
        yo = a_idft(1, rb)
        ye = ye_v[rows, :]
        out_v[rows, 0:DM] = jnp.concatenate([ye + yo, ye - yo], axis=1).astype(bf16)

    for c in c_wq:
        c.wait()

    qscale = np.float32(DH ** -0.5 * math.log2(math.e))

    def q_pair(j, carry):
        w = wq_v[j]
        wqp_v[0:DM, 0:DH] = _lo(w).astype(bf16)
        wqp_v[0:DM, DH:2 * DH] = _hi(w).astype(bf16)
        q = jnp.dot(x_v[...], wqp_v[...], preferred_element_type=f32) * qscale
        q_v[j] = q.astype(bf16)
        acc_v[pl.ds(pl.multiple_of(j * 64, 64), 64), :] = jnp.zeros((64, SEQ), f32)
        return carry

    lax.fori_loop(0, 8, q_pair, 0)

    def relayout(head):
        j = head // 2
        sh = ((1 - head % 2) * 16).astype(u32)
        for c0 in range(0, DC, 128):
            for n, src in enumerate((uk_v, uv_v)):
                w = src[j, c0:c0 + 128, :]
                wkv_v[c0:c0 + 128, n * DH:(n + 1) * DH] = pltpu.bitcast((w << sh) & HI16, f32).astype(bf16)

    def kv_rows(r0, k_dst, v_dst):
        kv = jnp.dot(ckv_v[r0:r0 + BQ, :], wkv_v[...], preferred_element_type=f32)
        k_dst[...] = kv[:, :DH].astype(bf16)
        v_dst[...] = kv[:, DH:].astype(bf16)

    c_ckv.wait()
    c_uk[0].wait()
    c_uv[0].wait()
    relayout(jnp.int32(0))
    kv_rows(0, kn_v, vn_v)
    c_wo.wait()
    for j in range(1, 8):
        c_uk[j].wait()
        c_uv[j].wait()

    def head(h, carry):
        qcol = pl.ds(pl.multiple_of((h % 2) * DH, DH), DH)
        ss, os_ = {}, {}
        for op, i in _head_schedule():
            r0 = i * BQ
            if op == "CP":
                k_v[0:BQ, :] = kn_v[...]
                v_v[0:BQ, :] = vn_v[...]
            elif op == "QK":
                ss[i] = _scores(q_v[h // 2, r0:r0 + BQ, qcol], k_v, r0)
            elif op == "PV":
                os_[i] = _context(*_softmax(*ss.pop(i), r0), v_v, r0)
            elif op == "KV":
                kv_rows(r0, k_v.at[r0:r0 + BQ], v_v.at[r0:r0 + BQ])
            elif op == "RL":
                relayout(jnp.minimum(h + 1, H - 1))
            elif op == "KVN":
                kv_rows(0, kn_v, vn_v)
            elif op == "O":
                t = lax.dot_general(wo_v[h], os_.pop(i), NT, preferred_element_type=f32)
                acc_v[64:512, r0:r0 + BQ] += t
        return carry

    lax.fori_loop(0, H, head, 0)

    def finalize(i, carry):
        rows = pl.ds(pl.multiple_of(i * BQ, BQ), BQ)
        lane = lax.broadcasted_iota(jnp.int32, (BQ, 128), 1)
        b = acc_v[:, rows].astype(bf16).T
        a_tail = jnp.where(lane < 64, out_v[rows, 384:512], jnp.zeros((BQ, 128), bf16))
        out_v[rows, 384:512] = jnp.where(lane < 64, a_tail, b[:, :128])
        out_v[rows, 512:896] = b[:, 128:]
        cp(out_v.at[rows], out_h.at[rows], sem.at[S_OUT + i]).start()
        return carry

    lax.fori_loop(0, NB, finalize, 0)
    for i in range(NB):
        r0 = i * BQ
        cp(out_v.at[r0:r0 + BQ], out_h.at[r0:r0 + BQ], sem.at[S_OUT + i]).wait()


@jax.jit
def pallas_concat_heads__spectral_gfnet__compressed_kv_cla__prompt_kernel(
    A_x: jax.Array,
    A_w_r: jax.Array,
    A_w_i: jax.Array,
    B_x: jax.Array,
    B_c_kv: jax.Array,
    B_w_q: jax.Array,
    B_w_uk: jax.Array,
    B_w_uv: jax.Array,
    B_w_o: jax.Array,
):
    fd, sf, si, gd = _dft_constants()
    args = (
        A_x.reshape(SEQ, DM).T,
        A_w_r.T,
        A_w_i.T,
        B_x.reshape(SEQ, DM).T,
        B_c_kv.reshape(SEQ, DC),
        B_w_q,
        B_w_uk,
        B_w_uv,
        jnp.transpose(B_w_o, (0, 2, 1)),
        fd, sf, si, gd,
    )
    vm = pltpu.VMEM
    scratch = [
        vm((DM, SEQ), bf16),
        vm((NF, SEQ), bf16),
        vm((NF, SEQ), bf16),
        vm((DM, SEQ), bf16),
        vm((SEQ, DC), bf16),
        vm((8, DM, DH), u32),
        vm((8, DC, DH), u32),
        vm((8, DC, DH), u32),
        vm((H, DM, DH), bf16),
        vm((2, 256, 256), bf16),
        vm((N1, 128, 128), bf16),
        vm((N1, 128, 128), bf16),
        vm((2, 256, 256), bf16),
        vm((2, SEQ, 256), bf16),
        vm((2, 2, SEQ, 128), f32),
        vm((2, 2, WP * N2, 128), f32),
        vm((SEQ, DM // 2), f32),
        vm((SEQ, 512), bf16),
        vm((512, 512), bf16),
        vm((8, SEQ, 2 * DH), bf16),
        vm((SEQ, DH), bf16),
        vm((SEQ, DH), bf16),
        vm((BQ, DH), bf16),
        vm((BQ, DH), bf16),
        vm((DC, 2 * DH), bf16),
        vm((512, SEQ), f32),
        vm((SEQ, 2 * DM), bf16),
        pltpu.SemaphoreType.DMA((N_SEM,)),
    ]
    out = pl.pallas_call(
        _kernel,
        in_specs=[pl.BlockSpec(memory_space=pl.ANY)] * len(args),
        out_specs=pl.BlockSpec(memory_space=pl.ANY),
        out_shape=jax.ShapeDtypeStruct((SEQ, 2 * DM), bf16),
        scratch_shapes=scratch,
        compiler_params=pltpu.CompilerParams(vmem_limit_bytes=120 * 2**20),
    )(*args)
    return out.reshape(1, SEQ, 2 * DM)
```

```python
import functools
import math

import jax
import jax.experimental.pallas as pl
import jax.experimental.pallas.tpu as pltpu
import jax.numpy as jnp
import numpy as np
from jax import lax

bf16 = jnp.bfloat16
f32 = jnp.float32
u32 = jnp.uint32
NT = (((1,), (1,)), ((), ()))

SEQ = 2048
DM = 448
NF = 225
H = 16
DH = 256
DC = 1024
BQ = 256
NB = SEQ // BQ
N1 = 32
N2 = 64
WP = N1 + 1
HI16 = np.uint32(0xFFFF0000)


def _to_bf16(a):
    return np.asarray(a, dtype=np.float32).astype(jnp.bfloat16)


@functools.lru_cache(maxsize=None)
def _dft_constants():
    half = DM // 2
    m = np.arange(half, dtype=np.float64)
    fd = np.zeros((2, 256, 256), np.float64)
    gd = np.zeros((2, 256, 256), np.float64)
    for par in range(2):
        ks = np.arange(par, NF, 2, dtype=np.float64)
        ang = 2.0 * np.pi * np.outer(m, ks) / DM
        nk = len(ks)
        fd[par, :half, :nk] = np.cos(ang)
        fd[par, :half, 128:128 + nk] = -np.sin(ang)
        wgt = np.full(nk, 2.0)
        wgt[(ks == 0) | (ks == half)] = 1.0
        gd[par, :nk, :half] = (np.cos(ang) * wgt / DM).T
        snk = -np.sin(ang) * wgt / DM
        snk[:, (ks == 0) | (ks == half)] = 0.0
        gd[par, 128:128 + nk, :half] = snk.T
    b = np.arange(N2, dtype=np.float64)
    sf = np.zeros((N1, 128, 128), np.float64)
    si = np.zeros((N1, 128, 128), np.float64)
    for f1 in range(N1):
        mat = np.exp(-2j * np.pi * (np.outer(b, b) / N2 + b[None, :] * f1 / SEQ))
        sf[f1] = np.block([[mat.real, -mat.imag], [mat.imag, mat.real]])
        inv = np.conj(mat).T / SEQ
        si[f1] = np.block([[inv.real, -inv.imag], [inv.imag, inv.real]])
    return _to_bf16(fd), _to_bf16(sf), _to_bf16(si), _to_bf16(gd)


def _lo(v):
    return pltpu.bitcast(v << 16, f32)


def _hi(v):
    return pltpu.bitcast(v & HI16, f32)


def _cmul_const(z, w):
    re, im = z
    c, s = w.real, w.imag
    if abs(s) < 1e-12:
        return (re, im) if c > 0 else (-re, -im)
    if abs(c) < 1e-12:
        return (-im, re) if s > 0 else (im, -re)
    if abs(abs(c) - abs(s)) < 1e-12:
        if c * s > 0:
            return ((re - im) * c, (re + im) * c)
        return ((re + im) * c, (im - re) * c)
    return (re * c - im * s, re * s + im * c)


def _fft(xs, sign):
    n = len(xs)
    if n == 1:
        return xs
    ev = _fft(xs[0::2], sign)
    od = _fft(xs[1::2], sign)
    out = [None] * n
    for k in range(n // 2):
        w = complex(math.cos(2 * math.pi * k / n), sign * math.sin(2 * math.pi * k / n))
        if 4 * k == n:
            tr, ti = od[k]
            if sign < 0:
                out[k] = (ev[k][0] + ti, ev[k][1] - tr)
                out[k + n // 2] = (ev[k][0] - ti, ev[k][1] + tr)
            else:
                out[k] = (ev[k][0] - ti, ev[k][1] + tr)
                out[k + n // 2] = (ev[k][0] + ti, ev[k][1] - tr)
            continue
        tr, ti = _cmul_const(od[k], w)
        out[k] = (ev[k][0] + tr, ev[k][1] + ti)
        out[k + n // 2] = (ev[k][0] - tr, ev[k][1] - ti)
    return out


def _radix32(ure, uim, rows, sign):
    for q in range(4):
        xs = [(ure[rows(4 * p + q), :], uim[rows(4 * p + q), :]) for p in range(8)]
        ys = _fft(xs, sign)
        for u in range(8):
            w = complex(math.cos(2 * math.pi * q * u / 32), sign * math.sin(2 * math.pi * q * u / 32))
            tr, ti = _cmul_const(ys[u], w)
            ure[rows(4 * u + q), :] = tr
            uim[rows(4 * u + q), :] = ti
    for u in range(8):
        xs = [(ure[rows(4 * u + q), :], uim[rows(4 * u + q), :]) for q in range(4)]
        ys = _fft(xs, sign)
        for v in range(4):
            ure[rows(4 * u + v), :] = ys[v][0]
            uim[rows(4 * u + v), :] = ys[v][1]


def _radix32_inv(ure, uim, rows, sign):
    for u in range(8):
        xs = [(ure[rows(4 * u + v), :], uim[rows(4 * u + v), :]) for v in range(4)]
        ys = _fft(xs, sign)
        for q in range(4):
            w = complex(math.cos(2 * math.pi * q * u / 32), sign * math.sin(2 * math.pi * q * u / 32))
            tr, ti = _cmul_const(ys[q], w)
            ure[rows(4 * u + q), :] = tr
            uim[rows(4 * u + q), :] = ti
    for q in range(4):
        xs = [(ure[rows(4 * u + q), :], uim[rows(4 * u + q), :]) for u in range(8)]
        ys = _fft(xs, sign)
        for p in range(8):
            ure[rows(4 * p + q), :] = ys[p][0]
            uim[rows(4 * p + q), :] = ys[p][1]


def _tri():
    r = lax.broadcasted_iota(jnp.int32, (128, 128), 0)
    c = lax.broadcasted_iota(jnp.int32, (128, 128), 1)
    return c <= r


def _scores(q, k_ref, r0):
    n = r0 + 128
    s = lax.dot_general(q, k_ref[0:n, :], NT, preferred_element_type=f32)
    se = lax.dot_general(q[128:], k_ref[n:n + 128, :], NT, preferred_element_type=f32)
    return s, se


def _softmax(s, se, r0):
    n = r0 + 128
    tri = _tri()
    p_rows, pe_rows, ls = [], [], []
    for rc in range(0, BQ, 16):
        tiles = [s[rc:rc + 16, c:c + 128] for c in range(0, n, 128)]
        if rc < 128:
            tiles[-1] = jnp.where(tri[rc:rc + 16], tiles[-1], -1e9)
        else:
            tiles.append(jnp.where(tri[rc - 128:rc - 112], se[rc - 128:rc - 112], -1e9))
        m = functools.reduce(jnp.maximum, tiles)
        m = jnp.max(m, axis=-1, keepdims=True)
        ps, l = [], None
        for x in tiles:
            p = jnp.exp2(x - m)
            l = p if l is None else l + p
            ps.append(p.astype(bf16))
        ls.append(jnp.sum(l, axis=-1, keepdims=True))
        if rc >= 128:
            pe_rows.append(ps.pop())
        p_rows.append(jnp.concatenate(ps, axis=1) if len(ps) > 1 else ps[0])
    l = jnp.concatenate(ls, axis=0)
    return jnp.concatenate(p_rows, axis=0), jnp.concatenate(pe_rows, axis=0), l[:128], l[128:]


def _context(p, pe, lu, ll, v_ref, r0):
    n = r0 + 128
    o = jnp.dot(p, v_ref[0:n, :], preferred_element_type=f32)
    oe = jnp.dot(pe, v_ref[n:n + 128, :], preferred_element_type=f32)
    return jnp.concatenate([o[:128] / lu, (o[128:] + oe) / ll], axis=0).astype(bf16)


HEAD_SCHEDULE = (
    ("CP", 0, 0), ("KV", 256, 512), ("QK", 0, 0), ("QK", 1, 0), ("KV", 512, 768), ("PV", 0, 0),
    ("QK", 2, 0), ("PV", 1, 0), ("KV", 768, 1024), ("O", 0, 0), ("QK", 3, 0), ("PV", 2, 0),
    ("O", 1, 0), ("PV", 3, 0), ("KV", 1280, 1408), ("KV", 1024, 1152), ("KV", 1152, 1280), ("O", 2, 0),
    ("KV", 1408, 1536), ("QK", 4, 0), ("KV", 1536, 1664), ("QK", 5, 0), ("PV", 4, 0), ("O", 3, 0),
    ("KV", 1664, 1792), ("KV", 1792, 1920), ("KV", 1920, 2048), ("QK", 6, 0), ("PV", 5, 0), ("PV", 6, 0),
    ("RL", 0, 0), ("O", 4, 0), ("QK", 7, 0), ("O", 5, 0), ("PV", 7, 0), ("KVN", 0, 0),
    ("O", 7, 0), ("O", 6, 0),
)


(S_XA, S_FD, S_SF, S_WR, S_WI, S_SI, S_GD, S_XB, S_CKV, S_WO, S_OA) = range(11)
S_WQ = 11
S_UK = S_WQ + 8
S_UV = S_UK + 8
S_OUT = S_UV + 8
N_SEM = S_OUT + NB


def _kernel(
    xa_h, wr_h, wi_h, xb_h, ckv_h, wq_h, uk_h, uv_h, wo_h, fd_h, sf_h, si_h, gd_h,
    out_h,
    xa_v, wr_v, wi_v, xb_v, ckv_v, wq_v, uk_v, uv_v, wo_v, fd_v, sf_v, si_v, gd_v,
    xf_v, u_v, wn_v, ye_v, x_v, wqp_v, q_v, k_v, v_v, kn_v, vn_v, wkv_v, acc_v, out_v, sem,
):
    cp = pltpu.make_async_copy
    wq_u, uk_u, uv_u = wq_h.bitcast(u32), uk_h.bitcast(u32), uv_h.bitcast(u32)
    c_xa = cp(xa_h, xa_v, sem.at[S_XA])
    c_fd = cp(fd_h, fd_v, sem.at[S_FD])
    c_sf = cp(sf_h, sf_v, sem.at[S_SF])
    c_wr = cp(wr_h, wr_v, sem.at[S_WR])
    c_wi = cp(wi_h, wi_v, sem.at[S_WI])
    c_si = cp(si_h, si_v, sem.at[S_SI])
    c_gd = cp(gd_h, gd_v, sem.at[S_GD])
    c_xb = cp(xb_h, xb_v, sem.at[S_XB])
    c_ckv = cp(ckv_h, ckv_v, sem.at[S_CKV])
    c_wo = cp(wo_h, wo_v, sem.at[S_WO])
    c_wq = [cp(wq_u.at[:, j, :], wq_v.at[j], sem.at[S_WQ + j]) for j in range(8)]
    c_uk = [cp(uk_u.at[:, j, :], uk_v.at[j], sem.at[S_UK + j]) for j in range(8)]
    c_uv = [cp(uv_u.at[:, j, :], uv_v.at[j], sem.at[S_UV + j]) for j in range(8)]
    for c in [c_xa, c_fd, c_wr, c_wi, c_sf, c_si, c_gd, c_xb] + c_wq + [c_ckv, c_uk[0], c_uv[0], c_wo]:
        c.start()
    for j in range(1, 8):
        c_uk[j].start()
        c_uv[j].start()

    half = DM // 2
    c_xa.wait()
    c_fd.wait()

    def a_fold(par):
        for cb in range(SEQ // 256):
            cols = slice(cb * 256, (cb + 1) * 256)
            x0 = xa_v[0:half, cols].astype(f32)
            x1 = xa_v[half:DM, cols].astype(f32)
            xf = (x0 + x1 if par == 0 else x0 - x1).astype(bf16)
            xf = jnp.concatenate([xf, jnp.zeros((256 - half, 256), bf16)], axis=0)
            xf_v[par, cols, :] = xf.T

    def a_dft(par):
        for rb in range(SEQ // 512):
            rows = slice(rb * 512, (rb + 1) * 512)
            u = jnp.dot(xf_v[par, rows, :], fd_v[par], preferred_element_type=f32)
            u_v[par, 0, rows, :] = u[:, :128]
            u_v[par, 1, rows, :] = u[:, 128:]

    def a_filter_prep(par):
        for ri, w_v in enumerate((wr_v, wi_v)):
            for cb in range(SEQ // 256):
                cols = slice(cb * 256, (cb + 1) * 256)
                wu = pltpu.bitcast(w_v[0:half, cols], u32)
                if par == 0:
                    last = w_v[half:NF, cols].astype(f32)
                    row0 = lax.broadcasted_iota(jnp.int32, (16, 256), 0) == 0
                    tail = jnp.where(row0, jnp.broadcast_to(last, (16, 256)), 0.0)
                    w = jnp.concatenate([_lo(wu), tail], axis=0).astype(bf16)
                else:
                    w = jnp.concatenate([_hi(wu), jnp.zeros((16, 256), f32)], axis=0).astype(bf16)
                wt = w.T.astype(f32)
                for g in range(256 // N1):
                    r0 = WP * (cb * (256 // N1) + g)
                    wn_v[par, ri, r0:r0 + N1, :] = wt[g * N1:(g + 1) * N1]

    def a_mid(par):
        for f1 in range(N1):
            slot = 4 * (f1 % 8) + f1 // 8
            rows = slice(slot * N2, (slot + 1) * N2)
            y = jnp.concatenate([u_v[par, 0, rows, :], u_v[par, 1, rows, :]], axis=0).astype(bf16)
            xs = jnp.dot(sf_v[f1], y, preferred_element_type=f32)
            xr, xi = xs[:N2], xs[N2:]
            fr = pl.ds(f1, N2, stride=WP)
            wr = wn_v[par, 0, fr, :]
            wi = wn_v[par, 1, fr, :]
            xw = jnp.concatenate([xr * wr - xi * wi, xr * wi + xi * wr], axis=0).astype(bf16)
            z = jnp.dot(si_v[f1], xw, preferred_element_type=f32)
            u_v[par, 0, rows, :] = z[:N2]
            u_v[par, 1, rows, :] = z[N2:]

    def a_radix(par, fn, sign):
        for r in range(0, N2, 8):
            fn(u_v.at[par, 0], u_v.at[par, 1], lambda blk: slice(blk * N2 + r, blk * N2 + r + 8), sign)

    def a_idft(par, rb):
        rows = slice(rb * 512, (rb + 1) * 512)
        z = jnp.concatenate([u_v[par, 0, rows, :], u_v[par, 1, rows, :]], axis=1).astype(bf16)
        return jnp.dot(z, gd_v[par], preferred_element_type=f32)[:, :half]

    for par in range(2):
        a_fold(par)
        a_dft(par)
    a_radix(0, _radix32, -1)
    for c in (c_wr, c_wi, c_sf, c_si):
        c.wait()
    a_filter_prep(0)
    a_filter_prep(1)
    a_radix(1, _radix32, -1)
    a_mid(0)
    a_radix(0, _radix32_inv, 1)
    a_mid(1)
    c_gd.wait()
    c_xb.wait()
    a_radix(1, _radix32_inv, 1)
    for cb in range(SEQ // 256):
        cols = slice(cb * 256, (cb + 1) * 256)
        x_v[cols, :] = jnp.concatenate([xb_v[:, cols], jnp.zeros((512 - DM, 256), bf16)], axis=0).T
    wqp_v[DM:512, :] = jnp.zeros((512 - DM, 512), bf16)
    for rb in range(SEQ // 512):
        ye_v[rb * 512:(rb + 1) * 512, :] = a_idft(0, rb)
    for rb in range(SEQ // 512):
        rows = slice(rb * 512, (rb + 1) * 512)
        yo = a_idft(1, rb)
        ye = ye_v[rows, :]
        out_v[rows, 0:DM] = jnp.concatenate([ye + yo, ye - yo], axis=1).astype(bf16)

    c_oa = cp(out_v.at[:, 0:384], out_h.at[:, 0:384], sem.at[S_OA])
    c_oa.start()

    for c in c_wq:
        c.wait()

    qscale = np.float32(DH ** -0.5 * math.log2(math.e))

    def q_pair(j, carry):
        w = wq_v[j]
        wqp_v[0:DM, 0:DH] = _lo(w).astype(bf16)
        wqp_v[0:DM, DH:2 * DH] = _hi(w).astype(bf16)
        q = jnp.dot(x_v[...], wqp_v[...], preferred_element_type=f32) * qscale
        q_v[j] = q.astype(bf16)
        acc_v[pl.ds(pl.multiple_of(j * 64, 64), 64), :] = jnp.zeros((64, SEQ), f32)
        return carry

    lax.fori_loop(0, 8, q_pair, 0)

    def relayout(head):
        j = head // 2
        sh = ((1 - head % 2) * 16).astype(u32)
        for c0 in range(0, DC, 128):
            for n, src in enumerate((uk_v, uv_v)):
                w = src[j, c0:c0 + 128, :]
                wkv_v[c0:c0 + 128, n * DH:(n + 1) * DH] = pltpu.bitcast((w << sh) & HI16, f32).astype(bf16)

    def kv_rows(r0, r1, k_dst, v_dst):
        kv = jnp.dot(ckv_v[r0:r1, :], wkv_v[...], preferred_element_type=f32)
        k_dst[...] = kv[:, :DH].astype(bf16)
        v_dst[...] = kv[:, DH:].astype(bf16)

    c_ckv.wait()
    c_uk[0].wait()
    c_uv[0].wait()
    relayout(jnp.int32(0))
    kv_rows(0, BQ, kn_v, vn_v)
    c_wo.wait()
    for j in range(1, 8):
        c_uk[j].wait()
        c_uv[j].wait()

    def head(h, carry):
        qcol = pl.ds(pl.multiple_of((h % 2) * DH, DH), DH)
        ss, os_ = {}, {}
        for op, i, i1 in HEAD_SCHEDULE:
            r0 = i * BQ
            if op == "CP":
                k_v[0:BQ, :] = kn_v[...]
                v_v[0:BQ, :] = vn_v[...]
            elif op == "QK":
                ss[i] = _scores(q_v[h // 2, r0:r0 + BQ, qcol], k_v, r0)
            elif op == "PV":
                os_[i] = _context(*_softmax(*ss.pop(i), r0), v_v, r0)
            elif op == "KV":
                kv_rows(i, i1, k_v.at[i:i1], v_v.at[i:i1])
            elif op == "RL":
                relayout(jnp.minimum(h + 1, H - 1))
            elif op == "KVN":
                kv_rows(0, BQ, kn_v, vn_v)
            elif op == "O":
                t = lax.dot_general(wo_v[h], os_.pop(i), NT, preferred_element_type=f32)
                acc_v[64:512, r0:r0 + BQ] += t
        return carry

    lax.fori_loop(0, H, head, 0)

    def finalize(i, carry):
        rows = pl.ds(pl.multiple_of(i * BQ, BQ), BQ)
        lane = lax.broadcasted_iota(jnp.int32, (BQ, 128), 1)
        b = acc_v[:, rows].astype(bf16).T
        a_tail = jnp.where(lane < 64, out_v[rows, 384:512], jnp.zeros((BQ, 128), bf16))
        out_v[rows, 384:512] = jnp.where(lane < 64, a_tail, b[:, :128])
        out_v[rows, 512:896] = b[:, 128:]
        cp(out_v.at[rows, 384:896], out_h.at[rows, 384:896], sem.at[S_OUT + i]).start()
        return carry

    lax.fori_loop(0, NB, finalize, 0)
    for i in range(NB):
        r0 = i * BQ
        cp(out_v.at[r0:r0 + BQ, 384:896], out_h.at[r0:r0 + BQ, 384:896], sem.at[S_OUT + i]).wait()
    c_oa.wait()


@jax.jit
def pallas_concat_heads__spectral_gfnet__compressed_kv_cla__prompt_kernel(
    A_x: jax.Array,
    A_w_r: jax.Array,
    A_w_i: jax.Array,
    B_x: jax.Array,
    B_c_kv: jax.Array,
    B_w_q: jax.Array,
    B_w_uk: jax.Array,
    B_w_uv: jax.Array,
    B_w_o: jax.Array,
):
    fd, sf, si, gd = _dft_constants()
    args = (
        A_x.reshape(SEQ, DM).T,
        A_w_r.T,
        A_w_i.T,
        B_x.reshape(SEQ, DM).T,
        B_c_kv.reshape(SEQ, DC),
        B_w_q,
        B_w_uk,
        B_w_uv,
        jnp.transpose(B_w_o, (0, 2, 1)),
        fd, sf, si, gd,
    )
    vm = pltpu.VMEM
    scratch = [
        vm((DM, SEQ), bf16),
        vm((NF, SEQ), bf16),
        vm((NF, SEQ), bf16),
        vm((DM, SEQ), bf16),
        vm((SEQ, DC), bf16),
        vm((8, DM, DH), u32),
        vm((8, DC, DH), u32),
        vm((8, DC, DH), u32),
        vm((H, DM, DH), bf16),
        vm((2, 256, 256), bf16),
        vm((N1, 128, 128), bf16),
        vm((N1, 128, 128), bf16),
        vm((2, 256, 256), bf16),
        vm((2, SEQ, 256), bf16),
        vm((2, 2, SEQ, 128), f32),
        vm((2, 2, WP * N2, 128), f32),
        vm((SEQ, DM // 2), f32),
        vm((SEQ, 512), bf16),
        vm((512, 512), bf16),
        vm((8, SEQ, 2 * DH), bf16),
        vm((SEQ, DH), bf16),
        vm((SEQ, DH), bf16),
        vm((BQ, DH), bf16),
        vm((BQ, DH), bf16),
        vm((DC, 2 * DH), bf16),
        vm((512, SEQ), f32),
        vm((SEQ, 2 * DM), bf16),
        pltpu.SemaphoreType.DMA((N_SEM,)),
    ]
    out = pl.pallas_call(
        _kernel,
        in_specs=[pl.BlockSpec(memory_space=pl.ANY)] * len(args),
        out_specs=pl.BlockSpec(memory_space=pl.ANY),
        out_shape=jax.ShapeDtypeStruct((SEQ, 2 * DM), bf16),
        scratch_shapes=scratch,
        compiler_params=pltpu.CompilerParams(vmem_limit_bytes=120 * 2**20),
    )(*args)
    return out.reshape(1, SEQ, 2 * DM)
```

```python
import functools
import math

import jax
import jax.experimental.pallas as pl
import jax.experimental.pallas.tpu as pltpu
import jax.numpy as jnp
import numpy as np
from jax import lax

bf16 = jnp.bfloat16
f32 = jnp.float32
u32 = jnp.uint32
NT = (((1,), (1,)), ((), ()))

SEQ = 2048
DM = 448
NF = 225
H = 16
DH = 256
DC = 1024
BQ = 256
NB = SEQ // BQ
N1 = 32
N2 = 64
WP = N1 + 1
RG = 8
HI16 = np.uint32(0xFFFF0000)


def _to_bf16(a):
    return np.asarray(a, dtype=np.float32).astype(jnp.bfloat16)


@functools.lru_cache(maxsize=None)
def _dft_constants():
    half = DM // 2
    m = np.arange(half, dtype=np.float64)
    fd = np.zeros((2, 256, 256), np.float64)
    gd = np.zeros((2, 256, 256), np.float64)
    for par in range(2):
        ks = np.arange(par, NF, 2, dtype=np.float64)
        ang = 2.0 * np.pi * np.outer(m, ks) / DM
        nk = len(ks)
        fd[par, :half, :nk] = np.cos(ang)
        fd[par, :half, 128:128 + nk] = -np.sin(ang)
        wgt = np.full(nk, 2.0)
        wgt[(ks == 0) | (ks == half)] = 1.0
        gd[par, :nk, :half] = (np.cos(ang) * wgt / DM).T
        snk = -np.sin(ang) * wgt / DM
        snk[:, (ks == 0) | (ks == half)] = 0.0
        gd[par, 128:128 + nk, :half] = snk.T
    b = np.arange(N2, dtype=np.float64)
    sf = np.zeros((N1, 128, 128), np.float64)
    si = np.zeros((N1, 128, 128), np.float64)
    for f1 in range(N1):
        mat = np.exp(-2j * np.pi * (np.outer(b, b) / N2 + b[None, :] * f1 / SEQ))
        sf[f1] = np.block([[mat.real, -mat.imag], [mat.imag, mat.real]])
        inv = np.conj(mat).T / SEQ
        si[f1] = np.block([[inv.real, -inv.imag], [inv.imag, inv.real]])
    return _to_bf16(fd), _to_bf16(sf), _to_bf16(si), _to_bf16(gd)


def _lo(v):
    return pltpu.bitcast(v << 16, f32)


def _hi(v):
    return pltpu.bitcast(v & HI16, f32)


def _cmul_const(z, w):
    re, im = z
    c, s = w.real, w.imag
    if abs(s) < 1e-12:
        return (re, im) if c > 0 else (-re, -im)
    if abs(c) < 1e-12:
        return (-im, re) if s > 0 else (im, -re)
    if abs(abs(c) - abs(s)) < 1e-12:
        if c * s > 0:
            return ((re - im) * c, (re + im) * c)
        return ((re + im) * c, (im - re) * c)
    return (re * c - im * s, re * s + im * c)


def _fft(xs, sign):
    n = len(xs)
    if n == 1:
        return xs
    ev = _fft(xs[0::2], sign)
    od = _fft(xs[1::2], sign)
    out = [None] * n
    for k in range(n // 2):
        w = complex(math.cos(2 * math.pi * k / n), sign * math.sin(2 * math.pi * k / n))
        if 4 * k == n:
            tr, ti = od[k]
            if sign < 0:
                out[k] = (ev[k][0] + ti, ev[k][1] - tr)
                out[k + n // 2] = (ev[k][0] - ti, ev[k][1] + tr)
            else:
                out[k] = (ev[k][0] - ti, ev[k][1] + tr)
                out[k + n // 2] = (ev[k][0] + ti, ev[k][1] - tr)
            continue
        tr, ti = _cmul_const(od[k], w)
        out[k] = (ev[k][0] + tr, ev[k][1] + ti)
        out[k + n // 2] = (ev[k][0] - tr, ev[k][1] - ti)
    return out


def _radix32(ure, uim, rows, sign):
    for q in range(4):
        xs = [(ure[rows(4 * p + q), :], uim[rows(4 * p + q), :]) for p in range(8)]
        ys = _fft(xs, sign)
        for u in range(8):
            w = complex(math.cos(2 * math.pi * q * u / 32), sign * math.sin(2 * math.pi * q * u / 32))
            tr, ti = _cmul_const(ys[u], w)
            ure[rows(4 * u + q), :] = tr
            uim[rows(4 * u + q), :] = ti
    for u in range(8):
        xs = [(ure[rows(4 * u + q), :], uim[rows(4 * u + q), :]) for q in range(4)]
        ys = _fft(xs, sign)
        for v in range(4):
            ure[rows(4 * u + v), :] = ys[v][0]
            uim[rows(4 * u + v), :] = ys[v][1]


def _radix32_inv(ure, uim, rows, sign):
    for u in range(8):
        xs = [(ure[rows(4 * u + v), :], uim[rows(4 * u + v), :]) for v in range(4)]
        ys = _fft(xs, sign)
        for q in range(4):
            w = complex(math.cos(2 * math.pi * q * u / 32), sign * math.sin(2 * math.pi * q * u / 32))
            tr, ti = _cmul_const(ys[q], w)
            ure[rows(4 * u + q), :] = tr
            uim[rows(4 * u + q), :] = ti
    for q in range(4):
        xs = [(ure[rows(4 * u + q), :], uim[rows(4 * u + q), :]) for u in range(8)]
        ys = _fft(xs, sign)
        for p in range(8):
            ure[rows(4 * p + q), :] = ys[p][0]
            uim[rows(4 * p + q), :] = ys[p][1]


def _tri():
    r = lax.broadcasted_iota(jnp.int32, (128, 128), 0)
    c = lax.broadcasted_iota(jnp.int32, (128, 128), 1)
    return c <= r


def _scores(q, k_ref, r0):
    n = r0 + 128
    s = lax.dot_general(q, k_ref[0:n, :], NT, preferred_element_type=f32)
    se = lax.dot_general(q[128:], k_ref[n:n + 128, :], NT, preferred_element_type=f32)
    return s, se


def _softmax(s, se, r0):
    n = r0 + 128
    tri = _tri()
    p_rows, pe_rows, ls = [], [], []
    for rc in range(0, BQ, 16):
        tiles = [s[rc:rc + 16, c:c + 128] for c in range(0, n, 128)]
        if rc < 128:
            tiles[-1] = jnp.where(tri[rc:rc + 16], tiles[-1], -1e9)
        else:
            tiles.append(jnp.where(tri[rc - 128:rc - 112], se[rc - 128:rc - 112], -1e9))
        m = functools.reduce(jnp.maximum, tiles)
        m = jnp.max(m, axis=-1, keepdims=True)
        ps, l = [], None
        for x in tiles:
            p = jnp.exp2(x - m)
            l = p if l is None else l + p
            ps.append(p.astype(bf16))
        ls.append(jnp.sum(l, axis=-1, keepdims=True))
        if rc >= 128:
            pe_rows.append(ps.pop())
        p_rows.append(jnp.concatenate(ps, axis=1) if len(ps) > 1 else ps[0])
    l = jnp.concatenate(ls, axis=0)
    return jnp.concatenate(p_rows, axis=0), jnp.concatenate(pe_rows, axis=0), l[:128], l[128:]


def _context(p, pe, lu, ll, v_ref, r0):
    n = r0 + 128
    o = jnp.dot(p, v_ref[0:n, :], preferred_element_type=f32)
    oe = jnp.dot(pe, v_ref[n:n + 128, :], preferred_element_type=f32)
    return jnp.concatenate([o[:128] / lu, (o[128:] + oe) / ll], axis=0).astype(bf16)


HEAD_SCHEDULE = (
    ("CP", 0, 0), ("KV", 256, 512), ("QK", 0, 0), ("QK", 1, 0), ("KV", 512, 768), ("PV", 0, 0),
    ("QK", 2, 0), ("PV", 1, 0), ("KV", 768, 1024), ("O", 0, 0), ("QK", 3, 0), ("PV", 2, 0),
    ("O", 1, 0), ("PV", 3, 0), ("KV", 1280, 1408), ("KV", 1024, 1152), ("KV", 1152, 1280), ("O", 2, 0),
    ("KV", 1408, 1536), ("QK", 4, 0), ("KV", 1536, 1664), ("QK", 5, 0), ("PV", 4, 0), ("O", 3, 0),
    ("KV", 1664, 1792), ("KV", 1792, 1920), ("KV", 1920, 2048), ("QK", 6, 0), ("PV", 5, 0), ("PV", 6, 0),
    ("RL", 0, 0), ("O", 4, 0), ("QK", 7, 0), ("O", 5, 0), ("PV", 7, 0), ("KVN", 0, 0),
    ("O", 7, 0), ("O", 6, 0),
)


(S_XA, S_FD, S_SF, S_WR, S_WI, S_SI, S_GD, S_XB, S_CKV, S_WO, S_OA) = range(11)
S_WQ = 11
S_UK = S_WQ + 8
S_UV = S_UK + 8
S_OUT = S_UV + 8
N_SEM = S_OUT + NB


def _kernel(
    xa_h, wr_h, wi_h, xb_h, ckv_h, wq_h, uk_h, uv_h, wo_h, fd_h, sf_h, si_h, gd_h,
    out_h,
    xa_v, wr_v, wi_v, xb_v, ckv_v, wq_v, uk_v, uv_v, wo_v, fd_v, sf_v, si_v, gd_v,
    xf_v, u_v, wn_v, ye_v, x_v, wqp_v, q_v, k_v, v_v, kn_v, vn_v, wkv_v, acc_v, out_v, sem,
):
    cp = pltpu.make_async_copy
    wq_u, uk_u, uv_u = wq_h.bitcast(u32), uk_h.bitcast(u32), uv_h.bitcast(u32)
    c_xa = cp(xa_h, xa_v, sem.at[S_XA])
    c_fd = cp(fd_h, fd_v, sem.at[S_FD])
    c_sf = cp(sf_h, sf_v, sem.at[S_SF])
    c_wr = cp(wr_h, wr_v, sem.at[S_WR])
    c_wi = cp(wi_h, wi_v, sem.at[S_WI])
    c_si = cp(si_h, si_v, sem.at[S_SI])
    c_gd = cp(gd_h, gd_v, sem.at[S_GD])
    c_xb = cp(xb_h, xb_v, sem.at[S_XB])
    c_ckv = cp(ckv_h, ckv_v, sem.at[S_CKV])
    c_wo = cp(wo_h, wo_v, sem.at[S_WO])
    c_wq = [cp(wq_u.at[:, j, :], wq_v.at[j], sem.at[S_WQ + j]) for j in range(8)]
    c_uk = [cp(uk_u.at[:, j, :], uk_v.at[j], sem.at[S_UK + j]) for j in range(8)]
    c_uv = [cp(uv_u.at[:, j, :], uv_v.at[j], sem.at[S_UV + j]) for j in range(8)]
    for c in [c_xa, c_fd, c_wr, c_wi, c_sf, c_si, c_gd, c_xb] + c_wq + [c_ckv, c_uk[0], c_uv[0], c_wo]:
        c.start()
    for j in range(1, 8):
        c_uk[j].start()
        c_uv[j].start()

    half = DM // 2
    c_xa.wait()
    c_fd.wait()

    def a_fold(par):
        for cb in range(SEQ // 256):
            cols = slice(cb * 256, (cb + 1) * 256)
            x0 = xa_v[0:half, cols].astype(f32)
            x1 = xa_v[half:DM, cols].astype(f32)
            xf = (x0 + x1 if par == 0 else x0 - x1).astype(bf16)
            xf = jnp.concatenate([xf, jnp.zeros((256 - half, 256), bf16)], axis=0)
            xf_v[par, cols, :] = xf.T

    def a_dft(par):
        for rb in range(SEQ // 512):
            rows = slice(rb * 512, (rb + 1) * 512)
            u = jnp.dot(xf_v[par, rows, :], fd_v[par], preferred_element_type=f32)
            u_v[par, 0, rows, :] = u[:, :128]
            u_v[par, 1, rows, :] = u[:, 128:]

    def a_filter_prep(par):
        for ri, w_v in enumerate((wr_v, wi_v)):
            for cb in range(SEQ // 256):
                cols = slice(cb * 256, (cb + 1) * 256)
                wu = pltpu.bitcast(w_v[0:half, cols], u32)
                if par == 0:
                    last = w_v[half:NF, cols].astype(f32)
                    row0 = lax.broadcasted_iota(jnp.int32, (16, 256), 0) == 0
                    tail = jnp.where(row0, jnp.broadcast_to(last, (16, 256)), 0.0)
                    w = jnp.concatenate([_lo(wu), tail], axis=0).astype(bf16)
                else:
                    w = jnp.concatenate([_hi(wu), jnp.zeros((16, 256), f32)], axis=0).astype(bf16)
                wt = w.T.astype(f32)
                for g in range(256 // N1):
                    r0 = WP * (cb * (256 // N1) + g)
                    wn_v[par, ri, r0:r0 + N1, :] = wt[g * N1:(g + 1) * N1]

    def a_mid(par):
        for f1 in range(N1):
            slot = 4 * (f1 % 8) + f1 // 8
            rows = slice(slot * N2, (slot + 1) * N2)
            y = jnp.concatenate([u_v[par, 0, rows, :], u_v[par, 1, rows, :]], axis=0).astype(bf16)
            xs = jnp.dot(sf_v[f1], y, preferred_element_type=f32)
            xr, xi = xs[:N2], xs[N2:]
            fr = pl.ds(f1, N2, stride=WP)
            wr = wn_v[par, 0, fr, :]
            wi = wn_v[par, 1, fr, :]
            xw = jnp.concatenate([xr * wr - xi * wi, xr * wi + xi * wr], axis=0).astype(bf16)
            z = jnp.dot(si_v[f1], xw, preferred_element_type=f32)
            u_v[par, 0, rows, :] = z[:N2]
            u_v[par, 1, rows, :] = z[N2:]

    def a_radix(par, fn, sign):
        for r in range(0, N2, RG):
            fn(u_v.at[par, 0], u_v.at[par, 1], lambda blk: slice(blk * N2 + r, blk * N2 + r + RG), sign)

    def a_idft(par, rb):
        rows = slice(rb * 512, (rb + 1) * 512)
        z = jnp.concatenate([u_v[par, 0, rows, :], u_v[par, 1, rows, :]], axis=1).astype(bf16)
        return jnp.dot(z, gd_v[par], preferred_element_type=f32)[:, :half]

    for par in range(2):
        a_fold(par)
        a_dft(par)
    a_radix(0, _radix32, -1)
    for c in (c_wr, c_wi, c_sf, c_si):
        c.wait()
    a_filter_prep(0)
    a_filter_prep(1)
    a_radix(1, _radix32, -1)
    a_mid(0)
    a_radix(0, _radix32_inv, 1)
    a_mid(1)
    c_gd.wait()
    c_xb.wait()
    a_radix(1, _radix32_inv, 1)
    for cb in range(SEQ // 256):
        cols = slice(cb * 256, (cb + 1) * 256)
        x_v[cols, :] = jnp.concatenate([xb_v[:, cols], jnp.zeros((512 - DM, 256), bf16)], axis=0).T
    wqp_v[:, DM:512, :] = jnp.zeros((2, 512 - DM, 512), bf16)
    for rb in range(SEQ // 512):
        ye_v[rb * 512:(rb + 1) * 512, :] = a_idft(0, rb)
    for rb in range(SEQ // 512):
        rows = slice(rb * 512, (rb + 1) * 512)
        yo = a_idft(1, rb)
        ye = ye_v[rows, :]
        out_v[rows, 0:DM] = jnp.concatenate([ye + yo, ye - yo], axis=1).astype(bf16)

    c_oa = cp(out_v.at[:, 0:384], out_h.at[:, 0:384], sem.at[S_OA])
    c_oa.start()

    for c in c_wq:
        c.wait()

    qscale = np.float32(DH ** -0.5 * math.log2(math.e))

    def wq_unpack(j):
        w = wq_v[j]
        wqp_v[j % 2, 0:DM, 0:DH] = _lo(w).astype(bf16)
        wqp_v[j % 2, 0:DM, DH:2 * DH] = _hi(w).astype(bf16)

    wq_unpack(0)

    def q_pair(j, carry):
        q = jnp.dot(x_v[...], wqp_v[j % 2], preferred_element_type=f32) * qscale
        wq_unpack(jnp.where(j == 7, 0, j + 1))
        q_v[j] = q.astype(bf16)
        acc_v[pl.ds(pl.multiple_of(j * 64, 64), 64), :] = jnp.zeros((64, SEQ), f32)
        return carry

    lax.fori_loop(0, 8, q_pair, 0)

    def relayout(head):
        j = head // 2
        sh = ((1 - head % 2) * 16).astype(u32)
        for c0 in range(0, DC, 128):
            for n, src in enumerate((uk_v, uv_v)):
                w = src[j, c0:c0 + 128, :]
                wkv_v[c0:c0 + 128, n * DH:(n + 1) * DH] = pltpu.bitcast((w << sh) & HI16, f32).astype(bf16)

    def kv_rows(r0, r1, k_dst, v_dst):
        kv = jnp.dot(ckv_v[r0:r1, :], wkv_v[...], preferred_element_type=f32)
        k_dst[...] = kv[:, :DH].astype(bf16)
        v_dst[...] = kv[:, DH:].astype(bf16)

    c_ckv.wait()
    c_uk[0].wait()
    c_uv[0].wait()
    relayout(jnp.int32(0))
    kv_rows(0, BQ, kn_v, vn_v)
    c_wo.wait()
    for j in range(1, 8):
        c_uk[j].wait()
        c_uv[j].wait()

    def head(h, carry):
        qcol = pl.ds(pl.multiple_of((h % 2) * DH, DH), DH)
        ss, os_ = {}, {}
        for op, i, i1 in HEAD_SCHEDULE:
            r0 = i * BQ
            if op == "CP":
                k_v[0:BQ, :] = kn_v[...]
                v_v[0:BQ, :] = vn_v[...]
            elif op == "QK":
                ss[i] = _scores(q_v[h // 2, r0:r0 + BQ, qcol], k_v, r0)
            elif op == "PV":
                os_[i] = _context(*_softmax(*ss.pop(i), r0), v_v, r0)
            elif op == "KV":
                kv_rows(i, i1, k_v.at[i:i1], v_v.at[i:i1])
            elif op == "RL":
                relayout(jnp.minimum(h + 1, H - 1))
            elif op == "KVN":
                kv_rows(0, BQ, kn_v, vn_v)
            elif op == "O":
                t = lax.dot_general(wo_v[h], os_.pop(i), NT, preferred_element_type=f32)
                acc_v[64:512, r0:r0 + BQ] += t
        return carry

    lax.fori_loop(0, H, head, 0)

    def finalize(i, carry):
        rows = pl.ds(pl.multiple_of(i * BQ, BQ), BQ)
        lane = lax.broadcasted_iota(jnp.int32, (BQ, 128), 1)
        b = acc_v[:, rows].astype(bf16).T
        a_tail = jnp.where(lane < 64, out_v[rows, 384:512], jnp.zeros((BQ, 128), bf16))
        out_v[rows, 384:512] = jnp.where(lane < 64, a_tail, b[:, :128])
        out_v[rows, 512:896] = b[:, 128:]
        cp(out_v.at[rows, 384:896], out_h.at[rows, 384:896], sem.at[S_OUT + i]).start()
        return carry

    lax.fori_loop(0, NB, finalize, 0)
    for i in range(NB):
        r0 = i * BQ
        cp(out_v.at[r0:r0 + BQ, 384:896], out_h.at[r0:r0 + BQ, 384:896], sem.at[S_OUT + i]).wait()
    c_oa.wait()


@jax.jit
def pallas_concat_heads__spectral_gfnet__compressed_kv_cla__prompt_kernel(
    A_x: jax.Array,
    A_w_r: jax.Array,
    A_w_i: jax.Array,
    B_x: jax.Array,
    B_c_kv: jax.Array,
    B_w_q: jax.Array,
    B_w_uk: jax.Array,
    B_w_uv: jax.Array,
    B_w_o: jax.Array,
):
    fd, sf, si, gd = _dft_constants()
    args = (
        A_x.reshape(SEQ, DM).T,
        A_w_r.T,
        A_w_i.T,
        B_x.reshape(SEQ, DM).T,
        B_c_kv.reshape(SEQ, DC),
        B_w_q,
        B_w_uk,
        B_w_uv,
        jnp.transpose(B_w_o, (0, 2, 1)),
        fd, sf, si, gd,
    )
    vm = pltpu.VMEM
    scratch = [
        vm((DM, SEQ), bf16),
        vm((NF, SEQ), bf16),
        vm((NF, SEQ), bf16),
        vm((DM, SEQ), bf16),
        vm((SEQ, DC), bf16),
        vm((8, DM, DH), u32),
        vm((8, DC, DH), u32),
        vm((8, DC, DH), u32),
        vm((H, DM, DH), bf16),
        vm((2, 256, 256), bf16),
        vm((N1, 128, 128), bf16),
        vm((N1, 128, 128), bf16),
        vm((2, 256, 256), bf16),
        vm((2, SEQ, 256), bf16),
        vm((2, 2, SEQ, 128), f32),
        vm((2, 2, WP * N2, 128), f32),
        vm((SEQ, DM // 2), f32),
        vm((SEQ, 512), bf16),
        vm((2, 512, 512), bf16),
        vm((8, SEQ, 2 * DH), bf16),
        vm((SEQ, DH), bf16),
        vm((SEQ, DH), bf16),
        vm((BQ, DH), bf16),
        vm((BQ, DH), bf16),
        vm((DC, 2 * DH), bf16),
        vm((512, SEQ), f32),
        vm((SEQ, 2 * DM), bf16),
        pltpu.SemaphoreType.DMA((N_SEM,)),
    ]
    out = pl.pallas_call(
        _kernel,
        in_specs=[pl.BlockSpec(memory_space=pl.ANY)] * len(args),
        out_specs=pl.BlockSpec(memory_space=pl.ANY),
        out_shape=jax.ShapeDtypeStruct((SEQ, 2 * DM), bf16),
        scratch_shapes=scratch,
        compiler_params=pltpu.CompilerParams(vmem_limit_bytes=120 * 2**20),
    )(*args)
    return out.reshape(1, SEQ, 2 * DM)
```
